```python
import jax
import jax.numpy as jnp

def _softmax(x, axis=-1):
    return jax.nn.softmax(x, axis=axis)

def _gelu(x):
    return jax.nn.gelu(x, approximate=True)

def _silu(x):
    return jax.nn.silu(x)

def _sigmoid(x):
    return jax.nn.sigmoid(x)

def _layernorm(x, axis=-1, eps=1e-05):
    m = jnp.mean(x, axis=axis, keepdims=True)
    v = jnp.var(x, axis=axis, keepdims=True)
    return (x - m) / jnp.sqrt(v + eps)

def _scatter_add(tgt, idx, src, axis=0):
    return tgt.at[idx].add(src)

def _segment_sum(src, seg, n):
    return jax.ops.segment_sum(src, seg, n)

class _Rng:

    def __init__(self, key):
        self._k = key

    def _next(self):
        self._k, sub = jax.random.split(self._k)
        return sub

    def normal(self, shape):
        return jax.random.normal(self._next(), shape, dtype=jnp.bfloat16)

    def randint(self, lo, hi, shape):
        return jax.random.randint(self._next(), shape, lo, hi, dtype=jnp.int32)

    def uniform(self, shape, lo=0.0, hi=1.0):
        return jax.random.uniform(self._next(), shape, jnp.bfloat16, lo, hi)

    def permutation(self, n):
        return jax.random.permutation(self._next(), n)
kernel_name = 'adaLN_cond__compressed_kv_cla__dense_activation_relu__decode'

def setup_inputs():
    _rng = _Rng(jax.random.key(int.from_bytes(__import__("os").urandom(4), "little")))
    _w = lambda a: (lambda t: t.astype(jnp.bfloat16) if jnp.issubdtype(t.dtype, jnp.floating) else t)(jnp.asarray(a))

    def _A_setup():
        B, H, Sq, Sk, D, M = (8, 32, 1, 4096, 128, 512)
        Dc = 4 * D
        return {'x': _w((lambda *s: _rng.normal(s) * 0.05)(B, Sq, M)), 'c_kv': _w((lambda *s: _rng.normal(s) * 0.05)(B, Sk, Dc)), 'w_q': _w((lambda *s: _rng.normal(s) * 0.05)(M, H, D) * M ** (-0.5)), 'w_uk': _w((lambda *s: _rng.normal(s) * 0.05)(Dc, H, D) * Dc ** (-0.5)), 'w_uv': _w((lambda *s: _rng.normal(s) * 0.05)(Dc, H, D) * Dc ** (-0.5)), 'w_o': _w((lambda *s: _rng.normal(s) * 0.05)(H, D, M) * (H * D) ** (-0.5))}
    _A_in = _A_setup()

    def _B_setup():
        B, S, D, Dff = (8, 1, 512, 1792)
        return {'x': _w((lambda *s: _rng.normal(s) * 0.05)(B, S, D)), 'w1': _w((lambda *s: _rng.normal(s) * 0.05)(D, Dff)), 'w2': _w((lambda *s: _rng.normal(s) * 0.05)(Dff, D))}
    _B_in = _B_setup()
    return {'A_x': _A_in['x'], 'A_c_kv': _A_in['c_kv'], 'A_w_q': _A_in['w_q'], 'A_w_uk': _A_in['w_uk'], 'A_w_uv': _A_in['w_uv'], 'A_w_o': _A_in['w_o'], 'B_x': _B_in['x'], 'B_w1': _B_in['w1'], 'B_w2': _B_in['w2'], 'c': _w((lambda *s: _rng.normal(s) * 0.05)(8, 512)), 'w_mod': _w((lambda *s: _rng.normal(s) * 0.05)(512, 6 * 512) * 512 ** (-0.5))}

def reference(A_x, A_c_kv, A_w_q, A_w_uk, A_w_uv, A_w_o, B_x, B_w1, B_w2, c, w_mod):

    def _A_ref(x, c_kv, w_q, w_uk, w_uv, w_o):
        B, Sq, M = (x.shape[0], x.shape[1], x.shape[2])
        Sk = c_kv.shape[1]
        H, D = (w_q.shape[1], w_q.shape[2])
        q = jnp.einsum('bqm,mhd->bhqd', x, w_q)
        k = jnp.einsum('bkc,chd->bhkd', c_kv, w_uk)
        v = jnp.einsum('bkc,chd->bhkd', c_kv, w_uv)
        scores = jnp.einsum('bhqd,bhkd->bhqk', q, k) * D ** (-0.5)
        off = Sk - Sq
        qi = jnp.arange(Sq)[:, None]
        kj = jnp.arange(Sk)[None, :]
        cmask = kj <= qi + off
        scores = jnp.where(cmask[None, None], scores, -1000000000.0)
        p = _softmax(scores, axis=-1)
        ctx = jnp.einsum('bhqk,bhkd->bhqd', p, v)
        return jnp.einsum('bhqd,hdm->bqm', ctx, w_o)

    def _B_ref(x, w1, w2):
        h = jnp.einsum('bsd,df->bsf', x, w1)
        zero = jnp.zeros_like(h)
        h = jnp.maximum(h, zero)
        return jnp.einsum('bsf,fd->bsd', h, w2)
    x = A_x
    mod = (_silu(c) @ w_mod).reshape(c.shape[0], 6, 1, -1)
    sa, ca, ga, sb, cb, gb = (mod[:, 0].copy(), mod[:, 1].copy(), mod[:, 2].copy(), mod[:, 3].copy(), mod[:, 4].copy(), mod[:, 5].copy())
    h = _layernorm(x, axis=-1) * (1 + ca) + sa
    x = x + ga * _A_ref(h, A_c_kv, A_w_q, A_w_uk, A_w_uv, A_w_o)
    h = _layernorm(x, axis=-1) * (1 + cb) + sb
    x = x + gb * _B_ref(h, B_w1, B_w2)
    return x
```

```python
import jax
import jax.numpy as jnp
from jax import lax
import jax.experimental.pallas as pl
import jax.experimental.pallas.tpu as pltpu

F32 = jnp.float32
BF16 = jnp.bfloat16
NT = (((1,), (1,)), ((), ()))


def _layernorm(x, eps=1e-05):
    m = jnp.mean(x, axis=-1, keepdims=True)
    xc = x - m
    v = jnp.mean(xc * xc, axis=-1, keepdims=True)
    return xc / jnp.sqrt(v + eps)


def _head_pair(w_ref, j, n_rows, n_pairs):
    w32 = w_ref.bitcast(jnp.uint32)[pl.ds(j, n_rows, stride=n_pairs), :]
    lo = pltpu.bitcast(w32 << 16, F32).astype(BF16)
    hi = pltpu.bitcast(w32 & jnp.uint32(0xFFFF0000), F32).astype(BF16)
    return lo, hi


@jax.jit
def pallas_adaLN_cond__compressed_kv_cla__dense_activation_relu__decode_kernel(
    A_x: jax.Array,
    A_c_kv: jax.Array,
    A_w_q: jax.Array,
    A_w_uk: jax.Array,
    A_w_uv: jax.Array,
    A_w_o: jax.Array,
    B_x: jax.Array,
    B_w1: jax.Array,
    B_w2: jax.Array,
    c: jax.Array,
    w_mod: jax.Array,
):
    del B_x
    B, Sq, M = A_x.shape
    _, Sk, Dc = A_c_kv.shape
    _, H, D = A_w_q.shape
    Dff = B_w1.shape[1]
    assert Sq == 1
    P = H // 2
    scale = float(D) ** -0.5

    def kernel(x_hbm, c_hbm, wmod_hbm, wq_hbm, wuk_hbm, ckv_hbm, wuv_hbm, wo_hbm, w1_hbm, w2_hbm,
               out_ref,
               x_v, c_v, wmod_v, wq_v, wuk_v, ckv_v, wuv_v, wo_v, w1_v, w2_v,
               qabs_v, ctxc_v, sems):
        copies = {}

        def add(name, src, dst):
            copies[name] = pltpu.make_async_copy(src, dst, sems.at[len(copies)])

        add("c", c_hbm, c_v)
        add("x", x_hbm, x_v)
        add("wmod_a", wmod_hbm.at[:, pl.ds(0, 2 * M)], wmod_v.at[:, pl.ds(0, 2 * M)])
        add("wq", wq_hbm, wq_v)
        add("wuk", wuk_hbm, wuk_v)
        for b in range(B):
            add(f"ckv{b}", ckv_hbm.at[b], ckv_v.at[b])
        add("wuv", wuv_hbm, wuv_v)
        add("wo", wo_hbm, wo_v)
        add("wmod_b", wmod_hbm.at[:, pl.ds(2 * M, 4 * M)], wmod_v.at[:, pl.ds(2 * M, 4 * M)])
        add("w1", w1_hbm, w1_v)
        add("w2", w2_hbm, w2_v)
        for cp in copies.values():
            cp.start()

        copies["c"].wait()
        copies["x"].wait()
        cf = c_v[...].astype(F32)
        sc = (cf * jax.nn.sigmoid(cf)).astype(BF16)
        x = x_v[...].astype(F32)
        copies["wmod_a"].wait()
        mod_a = jnp.dot(sc, wmod_v[:, 0:2 * M], preferred_element_type=F32)
        h = (_layernorm(x) * (1.0 + mod_a[:, M:2 * M]) + mod_a[:, 0:M]).astype(BF16)

        copies["wq"].wait()
        qs = []
        for j in range(P):
            for w in _head_pair(wq_v, j, M, P):
                qs.append(jnp.dot(h, w, preferred_element_type=F32).astype(BF16))
        copies["wuk"].wait()
        for j in range(P):
            for i, w in enumerate(_head_pair(wuk_v, j, Dc, P)):
                hd = 2 * j + i
                qa = lax.dot_general(qs[hd], w, NT, preferred_element_type=F32) * scale
                qabs_v[:, hd, :] = qa

        def attend(b):
            kv = ckv_v[b]
            s = lax.dot_general(qabs_v[b].astype(BF16), kv, NT, preferred_element_type=F32)
            m = jnp.max(s, axis=-1, keepdims=True)
            p = jnp.exp(s - m)
            l = jnp.sum(p, axis=-1, keepdims=True)
            o = jnp.dot(p.astype(BF16), kv, preferred_element_type=F32)
            ctxc_v[b] = o / l

        for b in range(B):
            copies[f"ckv{b}"].wait()
            attend(b)

        copies["wuv"].wait()
        ctx = []
        for j in range(P):
            for i, w in enumerate(_head_pair(wuv_v, j, Dc, P)):
                hd = 2 * j + i
                ctx.append(jnp.dot(ctxc_v[:, hd, :].astype(BF16), w,
                                   preferred_element_type=F32).astype(BF16))
        ctx = jnp.concatenate(ctx, axis=-1)
        copies["wo"].wait()
        att = jnp.dot(ctx, wo_v[...], preferred_element_type=F32)
        copies["wmod_b"].wait()
        mod_b = jnp.dot(sc, wmod_v[:, 2 * M:6 * M], preferred_element_type=F32)
        x1 = x + mod_b[:, 0:M] * att
        h2 = (_layernorm(x1) * (1.0 + mod_b[:, 2 * M:3 * M]) + mod_b[:, M:2 * M]).astype(BF16)
        copies["w1"].wait()
        f = jnp.maximum(jnp.dot(h2, w1_v[...], preferred_element_type=F32), 0.0).astype(BF16)
        copies["w2"].wait()
        y = jnp.dot(f, w2_v[...], preferred_element_type=F32)
        out_ref[...] = (x1 + mod_b[:, 3 * M:4 * M] * y).astype(out_ref.dtype)

    any_spec = pl.BlockSpec(memory_space=pl.ANY)
    out = pl.pallas_call(
        kernel,
        out_shape=jax.ShapeDtypeStruct((B, M), A_x.dtype),
        in_specs=[any_spec] * 10,
        out_specs=pl.BlockSpec(memory_space=pltpu.VMEM),
        scratch_shapes=[
            pltpu.VMEM((B, M), BF16),
            pltpu.VMEM((B, M), BF16),
            pltpu.VMEM((M, 6 * M), BF16),
            pltpu.VMEM((M * H, D), BF16),
            pltpu.VMEM((Dc * H, D), BF16),
            pltpu.VMEM((B, Sk, Dc), BF16),
            pltpu.VMEM((Dc * H, D), BF16),
            pltpu.VMEM((H * D, M), BF16),
            pltpu.VMEM((M, Dff), BF16),
            pltpu.VMEM((Dff, M), BF16),
            pltpu.VMEM((B, H, Dc), F32),
            pltpu.VMEM((B, H, Dc), F32),
            pltpu.SemaphoreType.DMA((32,)),
        ],
        compiler_params=pltpu.CompilerParams(vmem_limit_bytes=100 * 1024 * 1024),
    )(
        A_x.reshape(B, M), c, w_mod,
        A_w_q.reshape(M * H, D), A_w_uk.reshape(Dc * H, D), A_c_kv,
        A_w_uv.reshape(Dc * H, D), A_w_o.reshape(H * D, M), B_w1, B_w2,
    )
    return out.reshape(B, Sq, M)
```

```python
import jax
import jax.numpy as jnp
from jax import lax
import jax.experimental.pallas as pl
import jax.experimental.pallas.tpu as pltpu

F32 = jnp.float32
BF16 = jnp.bfloat16
NT = (((1,), (1,)), ((), ()))


def _layernorm(x, eps=1e-05):
    m = jnp.mean(x, axis=-1, keepdims=True)
    xc = x - m
    v = jnp.mean(xc * xc, axis=-1, keepdims=True)
    return xc / jnp.sqrt(v + eps)


def _loop(n, body):
    lax.fori_loop(0, n, lambda i, carry: body(i), None)


def _heads_to_front(src_ref, dst_ref, chunk=16):
    def body(i):
        rows = pl.ds(pl.multiple_of(i * chunk, chunk), chunk)
        dst_ref[:, rows, :] = jnp.swapaxes(src_ref[rows], 0, 1)
    _loop(src_ref.shape[0] // chunk, body)


@jax.jit
def pallas_adaLN_cond__compressed_kv_cla__dense_activation_relu__decode_kernel(
    A_x: jax.Array,
    A_c_kv: jax.Array,
    A_w_q: jax.Array,
    A_w_uk: jax.Array,
    A_w_uv: jax.Array,
    A_w_o: jax.Array,
    B_x: jax.Array,
    B_w1: jax.Array,
    B_w2: jax.Array,
    c: jax.Array,
    w_mod: jax.Array,
):
    del B_x
    B, Sq, M = A_x.shape
    _, Sk, Dc = A_c_kv.shape
    _, H, D = A_w_q.shape
    Dff = B_w1.shape[1]
    assert Sq == 1 and M == Dc and B >= 2
    scale = float(D) ** -0.5
    w2_cuts = (0, Dff - 512, Dff - 128, Dff)
    n_w2 = len(w2_cuts) - 1

    def kernel(x_hbm, c_hbm, wmod_hbm, wq_hbm, wuk_hbm, ckv_hbm, wuv_hbm, wo_hbm, w1_hbm, w2_hbm,
               out_ref,
               x_v, c_v, wmod_v, wq_v, wuk_v, ckv_v, wuv_v, wo_v, w1_v, w2_v,
               wt_v, q_v, qabs_v, ctxc_v, ctx_v, y_v):

        def ffn_out(f, i):
            lo, hi = w2_cuts[i], w2_cuts[i + 1]
            y = jnp.dot(f[:, lo:hi], w2_v[lo:hi, :], preferred_element_type=F32)
            return y if i == 0 else y + y_v[...]

        def stream(sems, ckv_sems, w2_sems):
            cp_wmod, cp_c, cp_x, cp_wq, cp_wuk, cp_wuv, cp_wo, cp_w1 = (
                pltpu.make_async_copy(src, dst, sems.at[i])
                for i, (src, dst) in enumerate((
                    (wmod_hbm, wmod_v), (c_hbm, c_v), (x_hbm, x_v), (wq_hbm, wq_v),
                    (wuk_hbm, wuk_v), (wuv_hbm, wuv_v), (wo_hbm, wo_v), (w1_hbm, w1_v))))

            def cp_ckv(b):
                return pltpu.make_async_copy(ckv_hbm.at[b], ckv_v.at[b], ckv_sems.at[b])

            def cp_w2(i):
                rows = pl.ds(w2_cuts[i], w2_cuts[i + 1] - w2_cuts[i])
                return pltpu.make_async_copy(w2_hbm.at[rows], w2_v.at[rows], w2_sems.at[i])

            for cp in (cp_wmod, cp_c, cp_x, cp_wq, cp_wuk):
                cp.start()

            cp_wmod.wait()
            cp_c.wait()
            cp_x.wait()
            cf = c_v[...].astype(F32)
            sc = (cf * jax.nn.sigmoid(cf)).astype(BF16)
            x = x_v[...].astype(F32)
            mod = jnp.dot(sc, wmod_v[...], preferred_element_type=F32)
            sa, ca, ga, sb, cb, gb = (mod[:, i * M:(i + 1) * M] for i in range(6))
            h = (_layernorm(x) * (1.0 + ca) + sa).astype(BF16)

            cp_wq.wait()
            cp_ckv(0).start()
            _heads_to_front(wq_v, wt_v)
            for hd in range(H):
                q_v[hd] = jnp.dot(h, wt_v[hd], preferred_element_type=F32)
            cp_wuk.wait()
            cp_ckv(1).start()
            _heads_to_front(wuk_v, wt_v)
            for hd in range(H):
                qa = lax.dot_general(q_v[hd].astype(BF16), wt_v[hd], NT,
                                     preferred_element_type=F32)
                qabs_v[:, hd, :] = qa * scale

            def attend(b):
                cp_ckv(b).wait()
                pl.when(b < B - 2)(lambda: cp_ckv(jnp.minimum(b + 2, B - 1)).start())
                pl.when(b == B - 2)(lambda: cp_wuv.start())
                pl.when(b == B - 1)(lambda: cp_wo.start())
                kv = ckv_v[b]
                s = lax.dot_general(qabs_v[b].astype(BF16), kv, NT, preferred_element_type=F32)
                p = jnp.exp(s - jnp.max(s, axis=-1, keepdims=True))
                o = jnp.dot(p.astype(BF16), kv, preferred_element_type=F32)
                ctxc_v[b] = o / jnp.sum(p, axis=-1, keepdims=True)
            _loop(B, attend)

            cp_wuv.wait()
            cp_w1.start()
            for i in range(n_w2):
                cp_w2(i).start()
            _heads_to_front(wuv_v, wt_v)
            for hd in range(H):
                ctx_v[hd] = jnp.dot(ctxc_v[:, hd, :].astype(BF16), wt_v[hd],
                                    preferred_element_type=F32)
            cp_wo.wait()
            ctx = jnp.concatenate([ctx_v[hd] for hd in range(H)], axis=-1).astype(BF16)
            x1 = x + ga * jnp.dot(ctx, wo_v[...], preferred_element_type=F32)

            h2 = (_layernorm(x1) * (1.0 + cb) + sb).astype(BF16)
            cp_w1.wait()
            f = jnp.maximum(jnp.dot(h2, w1_v[...], preferred_element_type=F32), 0.0).astype(BF16)
            for i in range(n_w2 - 1):
                cp_w2(i).wait()
                y_v[...] = ffn_out(f, i)
            cp_w2(n_w2 - 1).wait()
            return x1, gb, f

        x1, gb, f = pl.run_scoped(
            stream,
            pltpu.SemaphoreType.DMA((8,)),
            pltpu.SemaphoreType.DMA((B,)),
            pltpu.SemaphoreType.DMA((n_w2,)),
        )
        out_ref[...] = (x1 + gb * ffn_out(f, n_w2 - 1)).astype(out_ref.dtype)

    operands = (A_x.reshape(B, M), c, w_mod, A_w_q, A_w_uk, A_c_kv,
                A_w_uv, A_w_o.reshape(H * D, M), B_w1, B_w2)
    out = pl.pallas_call(
        kernel,
        out_shape=jax.ShapeDtypeStruct((B, M), A_x.dtype),
        in_specs=[pl.BlockSpec(memory_space=pl.ANY)] * len(operands),
        out_specs=pl.BlockSpec(memory_space=pltpu.VMEM),
        scratch_shapes=[pltpu.VMEM(a.shape, a.dtype) for a in operands] + [
            pltpu.VMEM((H, Dc, D), A_w_q.dtype),
            pltpu.VMEM((H, B, D), F32),
            pltpu.VMEM((B, H, Dc), F32),
            pltpu.VMEM((B, H, Dc), F32),
            pltpu.VMEM((H, B, D), F32),
            pltpu.VMEM((B, M), F32),
        ],
        compiler_params=pltpu.CompilerParams(vmem_limit_bytes=100 * 1024 * 1024),
    )(*operands)
    return out.reshape(B, Sq, M)
```

```python
import jax
import jax.numpy as jnp
from jax import lax
import jax.experimental.pallas as pl
import jax.experimental.pallas.tpu as pltpu

F32 = jnp.float32
BF16 = jnp.bfloat16
NT = (((1,), (1,)), ((), ()))


def _layernorm(x, eps=1e-05):
    m = jnp.mean(x, axis=-1, keepdims=True)
    xc = x - m
    v = jnp.mean(xc * xc, axis=-1, keepdims=True)
    return xc / jnp.sqrt(v + eps)


def _loop(n, body):
    lax.fori_loop(0, n, lambda i, carry: body(i), None)


def _heads_to_front(src_ref, dst_ref, chunk=16):
    def body(i):
        rows = pl.ds(pl.multiple_of(i * chunk, chunk), chunk)
        dst_ref[:, rows, :] = jnp.swapaxes(src_ref[rows], 0, 1)
    _loop(src_ref.shape[0] // chunk, body)


@jax.jit
def pallas_adaLN_cond__compressed_kv_cla__dense_activation_relu__decode_kernel(
    A_x: jax.Array,
    A_c_kv: jax.Array,
    A_w_q: jax.Array,
    A_w_uk: jax.Array,
    A_w_uv: jax.Array,
    A_w_o: jax.Array,
    B_x: jax.Array,
    B_w1: jax.Array,
    B_w2: jax.Array,
    c: jax.Array,
    w_mod: jax.Array,
):
    del B_x
    B, Sq, M = A_x.shape
    _, Sk, Dc = A_c_kv.shape
    _, H, D = A_w_q.shape
    Dff = B_w1.shape[1]
    assert Sq == 1 and M == Dc and B >= 2
    scale = float(D) ** -0.5
    w2_cuts = (0, Dff - 512, Dff - 128, Dff)
    n_w2 = len(w2_cuts) - 1

    def kernel(x_hbm, c_hbm, wmod_hbm, wq_hbm, wuk_hbm, ckv_hbm, wuv_hbm, wo_hbm, w1_hbm, w2_hbm,
               out_ref,
               x_v, c_v, wmod_v, wq_v, wuk_v, ckv_v, wuv_v, wo_v, w1_v, w2_v,
               wt_v, q_v, qabs_v, ctxc_v, ctx_v, y_v):

        def ffn_out(f, i):
            lo, hi = w2_cuts[i], w2_cuts[i + 1]
            y = jnp.dot(f[:, lo:hi], w2_v[lo:hi, :], preferred_element_type=F32)
            return y if i == 0 else y + y_v[...]

        def stream(sems, ckv_sems, w2_sems):
            cp_wmod, cp_c, cp_x, cp_wq, cp_wuk, cp_wuv, cp_wo, cp_w1 = (
                pltpu.make_async_copy(src, dst, sems.at[i])
                for i, (src, dst) in enumerate((
                    (wmod_hbm, wmod_v), (c_hbm, c_v), (x_hbm, x_v), (wq_hbm, wq_v),
                    (wuk_hbm, wuk_v), (wuv_hbm, wuv_v), (wo_hbm, wo_v), (w1_hbm, w1_v))))

            def cp_ckv(b):
                return pltpu.make_async_copy(ckv_hbm.at[b], ckv_v.at[b], ckv_sems.at[b])

            def cp_w2(i):
                rows = pl.ds(w2_cuts[i], w2_cuts[i + 1] - w2_cuts[i])
                return pltpu.make_async_copy(w2_hbm.at[rows], w2_v.at[rows], w2_sems.at[i])

            for cp in (cp_wmod, cp_c, cp_x, cp_wq):
                cp.start()

            cp_wmod.wait()
            cp_c.wait()
            cp_x.wait()
            cp_wuk.start()
            cf = c_v[...].astype(F32)
            sc = (cf * jax.nn.sigmoid(cf)).astype(BF16)
            x = x_v[...].astype(F32)
            mod = jnp.dot(sc, wmod_v[...], preferred_element_type=F32)
            sa, ca, ga, sb, cb, gb = (mod[:, i * M:(i + 1) * M] for i in range(6))
            h = (_layernorm(x) * (1.0 + ca) + sa).astype(BF16)

            cp_wq.wait()
            cp_ckv(0).start()
            _heads_to_front(wq_v, wt_v)
            for hd in range(H):
                q_v[hd] = jnp.dot(h, wt_v[hd], preferred_element_type=F32)
            cp_wuk.wait()
            cp_ckv(1).start()
            _heads_to_front(wuk_v, wt_v)
            for hd in range(H):
                qa = lax.dot_general(q_v[hd].astype(BF16), wt_v[hd], NT,
                                     preferred_element_type=F32)
                qabs_v[:, hd, :] = qa * scale

            def attend(b):
                cp_ckv(b).wait()
                pl.when(b < B - 2)(lambda: cp_ckv(jnp.minimum(b + 2, B - 1)).start())
                pl.when(b == B - 2)(lambda: cp_wuv.start())
                pl.when(b == B - 1)(lambda: cp_wo.start())
                kv = ckv_v[b]
                s = lax.dot_general(qabs_v[b].astype(BF16), kv, NT, preferred_element_type=F32)
                p = jnp.exp(s - jnp.max(s, axis=-1, keepdims=True))
                o = jnp.dot(p.astype(BF16), kv, preferred_element_type=F32)
                ctxc_v[b] = o / jnp.sum(p, axis=-1, keepdims=True)
            _loop(B, attend)

            cp_wuv.wait()
            cp_w1.start()
            _heads_to_front(wuv_v, wt_v)
            for hd in range(H):
                ctx_v[hd] = jnp.dot(ctxc_v[:, hd, :].astype(BF16), wt_v[hd],
                                    preferred_element_type=F32)
            cp_wo.wait()
            cp_w2(0).start()
            ctx = jnp.concatenate([ctx_v[hd] for hd in range(H)], axis=-1).astype(BF16)
            x1 = x + ga * jnp.dot(ctx, wo_v[...], preferred_element_type=F32)

            h2 = (_layernorm(x1) * (1.0 + cb) + sb).astype(BF16)
            cp_w1.wait()
            for i in range(1, n_w2):
                cp_w2(i).start()
            f = jnp.maximum(jnp.dot(h2, w1_v[...], preferred_element_type=F32), 0.0).astype(BF16)
            for i in range(n_w2 - 1):
                cp_w2(i).wait()
                y_v[...] = ffn_out(f, i)
            cp_w2(n_w2 - 1).wait()
            return x1, gb, f

        x1, gb, f = pl.run_scoped(
            stream,
            pltpu.SemaphoreType.DMA((8,)),
            pltpu.SemaphoreType.DMA((B,)),
            pltpu.SemaphoreType.DMA((n_w2,)),
        )
        out_ref[...] = (x1 + gb * ffn_out(f, n_w2 - 1)).astype(out_ref.dtype)

    operands = (A_x.reshape(B, M), c, w_mod, A_w_q, A_w_uk, A_c_kv,
                A_w_uv, A_w_o.reshape(H * D, M), B_w1, B_w2)
    out = pl.pallas_call(
        kernel,
        out_shape=jax.ShapeDtypeStruct((B, M), A_x.dtype),
        in_specs=[pl.BlockSpec(memory_space=pl.ANY)] * len(operands),
        out_specs=pl.BlockSpec(memory_space=pltpu.VMEM),
        scratch_shapes=[pltpu.VMEM(a.shape, a.dtype) for a in operands] + [
            pltpu.VMEM((H, Dc, D), A_w_q.dtype),
            pltpu.VMEM((H, B, D), F32),
            pltpu.VMEM((B, H, Dc), F32),
            pltpu.VMEM((B, H, Dc), F32),
            pltpu.VMEM((H, B, D), F32),
            pltpu.VMEM((B, M), F32),
        ],
        compiler_params=pltpu.CompilerParams(vmem_limit_bytes=100 * 1024 * 1024),
    )(*operands)
    return out.reshape(B, Sq, M)
```
